```python
import jax
import jax.numpy as jnp

def _softmax(x, axis=-1):
    return jax.nn.softmax(x, axis=axis)

def _gelu(x):
    return jax.nn.gelu(x, approximate=True)

def _silu(x):
    return jax.nn.silu(x)

def _sigmoid(x):
    return jax.nn.sigmoid(x)

def _layernorm(x, axis=-1, eps=1e-05):
    m = jnp.mean(x, axis=axis, keepdims=True)
    v = jnp.var(x, axis=axis, keepdims=True)
    return (x - m) / jnp.sqrt(v + eps)

def _scatter_add(tgt, idx, src, axis=0):
    return tgt.at[idx].add(src)

def _segment_sum(src, seg, n):
    return jax.ops.segment_sum(src, seg, n)

class _Rng:

    def __init__(self, key):
        self._k = key

    def _next(self):
        self._k, sub = jax.random.split(self._k)
        return sub

    def normal(self, shape):
        return jax.random.normal(self._next(), shape, dtype=jnp.bfloat16)

    def randint(self, lo, hi, shape):
        return jax.random.randint(self._next(), shape, lo, hi, dtype=jnp.int32)

    def uniform(self, shape, lo=0.0, hi=1.0):
        return jax.random.uniform(self._next(), shape, jnp.bfloat16, lo, hi)

    def permutation(self, n):
        return jax.random.permutation(self._next(), n)
kernel_name = 'adaLN_cond__ssm_conv_h3__glu_gated_bilinear__prompt'

def setup_inputs():
    _rng = _Rng(jax.random.key(int.from_bytes(__import__("os").urandom(4), "little")))
    _w = lambda a: (lambda t: t.astype(jnp.bfloat16) if jnp.issubdtype(t.dtype, jnp.floating) else t)(jnp.asarray(a))

    def _A_setup():
        B, S, D = (1, 2048, 640)
        ks = 4
        return {'q': _w((lambda *s: _rng.normal(s) * 0.05)(B, S, D)), 'k': _w((lambda *s: _rng.normal(s) * 0.05)(B, S, D)), 'v': _w((lambda *s: _rng.normal(s) * 0.05)(B, S, D)), 'shift_k': _w((lambda *s: _rng.normal(s) * 0.05)(D, ks) * 0.5), 'ssm_k': _w((lambda *s: _rng.normal(s) * 0.05)(D, S) * (1.0 / S ** 0.5)), 'ssm_D': _w((lambda *s: _rng.normal(s) * 0.05)(D))}
    _A_in = _A_setup()

    def _B_setup():
        B, S, D, F = (1, 2048, 640, 1536)
        return {'x': _w((lambda *s: _rng.normal(s) * 0.05)(B, S, D)), 'w_gate': _w((lambda *s: _rng.normal(s) * 0.05)(D, F) * D ** (-0.5)), 'w_up': _w((lambda *s: _rng.normal(s) * 0.05)(D, F) * D ** (-0.5)), 'w_down': _w((lambda *s: _rng.normal(s) * 0.05)(F, D) * F ** (-0.5))}
    _B_in = _B_setup()
    return {'A_q': _A_in['q'], 'A_k': _A_in['k'], 'A_v': _A_in['v'], 'A_shift_k': _A_in['shift_k'], 'A_ssm_k': _A_in['ssm_k'], 'A_ssm_D': _A_in['ssm_D'], 'B_x': _B_in['x'], 'B_w_gate': _B_in['w_gate'], 'B_w_up': _B_in['w_up'], 'B_w_down': _B_in['w_down'], 'c': _w((lambda *s: _rng.normal(s) * 0.05)(1, 640)), 'w_mod': _w((lambda *s: _rng.normal(s) * 0.05)(640, 6 * 640) * 640 ** (-0.5))}

def reference(A_q, A_k, A_v, A_shift_k, A_ssm_k, A_ssm_D, B_x, B_w_gate, B_w_up, B_w_down, c, w_mod):

    def _A_ref(q, k, v, shift_k, ssm_k, ssm_D):
        B, S, D = q.shape
        ks = shift_k.shape[-1]
        k_pad = jnp.pad(k, ((0, 0), (ks - 1, 0), (0, 0)))
        k_shift = jnp.zeros_like(k)
        for t in range(ks):
            k_shift = k_shift + k_pad[:, t:t + S, :] * shift_k[:, ks - 1 - t][None, None, :]
        kv = k_shift * v
        L = 2 * S
        kv_pad = jnp.pad(kv, ((0, 0), (0, S), (0, 0)))
        kf_pad = jnp.pad(ssm_k, ((0, 0), (0, S)))
        kv_f = (lambda x, axes=(-2, -1): jnp.fft.rfft2(x.astype(jnp.float32), axes=axes))(kv_pad[:, None, :, :], axes=(1, 2))
        kf_f = (lambda x, axes=(-2, -1): jnp.fft.rfft2(x.astype(jnp.float32), axes=axes))(kf_pad[:, None, :], axes=(1, 2))
        kf_f = (lambda x, *d: x.transpose(*d))(kf_f, 1, 2, 0)
        y_f = kv_f * kf_f[None, :, :, :]
        y = (lambda x, s, axes=(-2, -1): jnp.fft.irfft2(x, s=s, axes=axes).astype(jnp.bfloat16))(y_f, (1, L), axes=(1, 2))[:, 0, :S, :]
        y = y + kv * ssm_D[None, None, :]
        return q * y

    def _B_ref(x, w_gate, w_up, w_down):
        g = jnp.einsum('bsd,df->bsf', x, w_gate)
        u = jnp.einsum('bsd,df->bsf', x, w_up)
        h = g * u
        return jnp.einsum('bsf,fd->bsd', h, w_down)
    x = A_q
    mod = (_silu(c) @ w_mod).reshape(c.shape[0], 6, 1, -1)
    sa, ca, ga, sb, cb, gb = (mod[:, 0].copy(), mod[:, 1].copy(), mod[:, 2].copy(), mod[:, 3].copy(), mod[:, 4].copy(), mod[:, 5].copy())
    h = _layernorm(x, axis=-1) * (1 + ca) + sa
    x = x + ga * _A_ref(h, A_k, A_v, A_shift_k, A_ssm_k, A_ssm_D)
    h = _layernorm(x, axis=-1) * (1 + cb) + sb
    x = x + gb * _B_ref(h, B_w_gate, B_w_up, B_w_down)
    return x
```

```python
import functools

import jax
import jax.numpy as jnp
import numpy as np
from jax.experimental import pallas as pl
from jax.experimental.pallas import tpu as pltpu

S, D, F, KS = 2048, 640, 1536, 4
C = 128
NC = S // C
MB = 256
NB = S // MB
EPS = 1e-5
F32 = jnp.float32
BF16 = jnp.bfloat16


def _dft_matrices():
    n = np.arange(C, dtype=np.float64)
    k = np.concatenate([np.arange(0, C, 2), np.arange(1, C, 2)]).astype(np.float64)
    theta = np.pi * np.outer(2.0 * k + 1.0, n) / (2.0 * C)
    fwd = np.concatenate([np.cos(theta), -np.sin(theta)], axis=0)
    inv = fwd.T / C
    return fwd.astype(np.float32), np.ascontiguousarray(inv).astype(np.float32)


_FWD, _INV = _dft_matrices()


def _layernorm(x):
    m = jnp.mean(x, axis=-1, keepdims=True)
    d = x - m
    v = jnp.mean(d * d, axis=-1, keepdims=True)
    return d * jax.lax.rsqrt(v + EPS)


def _kernel(q_hbm, k_hbm, v_hbm, sk_hbm, ssm_hbm, sd_hbm, wg_hbm, wu_hbm, wd_hbm, c_hbm, wm_hbm,
            fwd_hbm, inv_hbm,
            out_hbm,
            q_v, k_v, v_v, sk_v, ssm_v, sd_v, wg_v, wu_v, wd_v, c_v, wm_v, fwd_v, inv_v,
            kv_v, a_v, kf_v, w_v, y_v, mod_v, o_v, sems):

    copies = {}

    def plan(name, src, dst):
        copies[name] = pltpu.make_async_copy(src, dst, sems.at[len(copies)])

    plan("fwd", fwd_hbm, fwd_v)
    plan("sk", sk_hbm, sk_v)
    for j in range(NB):
        r = pl.ds(j * MB, MB)
        plan(("k", j), k_hbm.at[0, r, :], k_v.at[r, :])
        plan(("v", j), v_hbm.at[0, r, :], v_v.at[r, :])
        plan(("s", j), ssm_hbm.at[:, r], ssm_v.at[:, r])
        if j == 0:
            plan("inv", inv_hbm, inv_v)
            plan("sd", sd_hbm, sd_v)
    plan("c", c_hbm, c_v)
    plan("wm", wm_hbm, wm_v)
    plan("q", q_hbm.at[0], q_v)
    plan("wg", wg_hbm, wg_v)
    plan("wu", wu_hbm, wu_v)
    plan("wd", wd_hbm, wd_v)
    n_in = len(copies)
    for cp in copies.values():
        cp.start()
    out_copies = [
        pltpu.make_async_copy(o_v.at[pl.ds(j * MB, MB), :], out_hbm.at[0, pl.ds(j * MB, MB), :],
                              sems.at[n_in + j])
        for j in range(NB)
    ]

    def wait(*names):
        for nm in names:
            copies[nm].wait()

    wait("fwd", "sk")
    fwd = fwd_v[...]
    skt = sk_v[...].astype(F32).T
    tap = [jnp.broadcast_to(skt[j:j + 1, :], (8, D)) for j in range(KS)]

    def kv_chunk(c):
        r0 = c * C
        if c == 0:
            x = jnp.concatenate([jnp.zeros((16, D), F32), k_v[0:C, :].astype(F32)], axis=0)
        else:
            x = k_v[r0 - 16:r0 + C, :].astype(F32)
        ks = x[16:16 + C] * tap[0][0:1]
        for j in range(1, KS):
            ks = ks + pltpu.roll(x, j, 0)[16:16 + C] * tap[j][0:1]
        kv = (ks * v_v[r0:r0 + C, :].astype(F32)).astype(BF16)
        kv_v[r0:r0 + C, :] = kv
        return kv

    def signal_dft(c, kv):
        a = jnp.dot(fwd, kv, preferred_element_type=F32)
        a_v[c, 0] = a[:C]
        a_v[c, 1] = a[C:]
        a_v[c, 2] = a[:C] + a[C:]

    def filter_dft(p, prev):
        g = jax.lax.dot_general(fwd, ssm_v[:, p * C:(p + 1) * C], (((1,), (1,)), ((), ())),
                                preferred_element_type=F32)
        re, im = g[:C], g[C:]
        if prev is not None:
            pre, pim = prev
            h = C // 2
            re = jnp.concatenate([re[:h] - pim[:h], re[h:] + pim[h:]], axis=0)
            im = jnp.concatenate([im[:h] + pre[:h], im[h:] - pre[h:]], axis=0)
        kf_v[p, 0] = re
        kf_v[p, 1] = im
        kf_v[p, 2] = re + im
        return g[:C], g[C:]

    def mac(c0):
        G = 8
        for r in range(0, C, G):
            rows = pl.ds(r, G)
            acc = [[None] * 3, [None] * 3]
            prev_a = None
            for p in range(c0 + 1, -1, -1):
                kk = [kf_v[p, i, rows, :] for i in range(3)]
                cur_a = [a_v[c0 + 1 - p, i, rows, :] for i in range(3)]
                for i in range(3):
                    t = kk[i] * cur_a[i]
                    acc[1][i] = t if acc[1][i] is None else acc[1][i] + t
                if prev_a is not None:
                    for i in range(3):
                        t = kk[i] * prev_a[i]
                        acc[0][i] = t if acc[0][i] is None else acc[0][i] + t
                prev_a = cur_a
            for o in range(2):
                m1, m2, m3 = acc[o]
                w_v[o, pl.ds(r, G), :] = (m1 - m2).astype(BF16)
                w_v[o, pl.ds(C + r, G), :] = (m3 - m1 - m2).astype(BF16)

    def inverse_dft(c, o, sd):
        r0 = c * C
        y = jnp.dot(inv_v[...], w_v[o], preferred_element_type=F32)
        y_v[r0:r0 + C, :] = y + kv_v[r0:r0 + C, :].astype(F32) * sd

    prev = None
    sd = None
    for j in range(NB):
        wait(("k", j), ("v", j), ("s", j))
        for c in (2 * j, 2 * j + 1):
            signal_dft(c, kv_chunk(c))
            prev = filter_dft(c, prev)
        mac(2 * j)
        if j == 0:
            wait("inv", "sd")
            sd = sd_v[...].astype(F32)
        for o in range(2):
            inverse_dft(2 * j + o, o, sd)

    wait("c", "wm")
    cc = c_v[...].astype(F32)
    sc = (cc * jax.nn.sigmoid(cc)).astype(BF16)
    mod = jnp.dot(jnp.broadcast_to(sc, (16, D)), wm_v[...], preferred_element_type=F32)[0:8]
    sa, ca, ga, sb, cb, gb = (mod[:, i * D:(i + 1) * D] for i in range(6))
    mod_v[0] = ga * (1.0 + ca)
    mod_v[1] = ga * sa
    mod_v[2] = 1.0 + cb
    mod_v[3] = sb
    mod_v[4] = gb

    wait("q", "wg", "wu", "wd")
    FB = 512

    @pl.loop(0, NB)
    def _(j):
        rows = pl.ds(pl.multiple_of(j * MB, MB), MB)
        qq = q_v[rows, :].astype(F32)
        x = qq + y_v[rows, :] * (_layernorm(qq) * mod_v[0][0:1] + mod_v[1][0:1])
        h = (_layernorm(x) * mod_v[2][0:1] + mod_v[3][0:1]).astype(BF16)
        acc = None
        for f in range(0, F, FB):
            g = jnp.dot(h, wg_v[:, f:f + FB], preferred_element_type=F32)
            u = jnp.dot(h, wu_v[:, f:f + FB], preferred_element_type=F32)
            t = jnp.dot((g * u).astype(BF16), wd_v[f:f + FB, :], preferred_element_type=F32)
            acc = t if acc is None else acc + t
        o_v[rows, :] = (x + acc * mod_v[4][0:1]).astype(BF16)

    for cp in out_copies:
        cp.start()
    for cp in out_copies:
        cp.wait()


@jax.jit
def pallas_adaLN_cond__ssm_conv_h3__glu_gated_bilinear__prompt_kernel(
    A_q: jax.Array,
    A_k: jax.Array,
    A_v: jax.Array,
    A_shift_k: jax.Array,
    A_ssm_k: jax.Array,
    A_ssm_D: jax.Array,
    B_x: jax.Array,
    B_w_gate: jax.Array,
    B_w_up: jax.Array,
    B_w_down: jax.Array,
    c: jax.Array,
    w_mod: jax.Array,
):
    del B_x
    any_spec = pl.BlockSpec(memory_space=pl.ANY)
    n_dma = 2 + 3 * NB + 2 + 6 + NB
    return pl.pallas_call(
        _kernel,
        out_shape=jax.ShapeDtypeStruct((1, S, D), BF16),
        in_specs=[any_spec] * 13,
        out_specs=any_spec,
        scratch_shapes=[
            pltpu.VMEM((S, D), BF16),
            pltpu.VMEM((S, D), BF16),
            pltpu.VMEM((S, D), BF16),
            pltpu.VMEM((D, KS), BF16),
            pltpu.VMEM((D, S), BF16),
            pltpu.VMEM((1, D), BF16),
            pltpu.VMEM((D, F), BF16),
            pltpu.VMEM((D, F), BF16),
            pltpu.VMEM((F, D), BF16),
            pltpu.VMEM((1, D), BF16),
            pltpu.VMEM((D, 6 * D), BF16),
            pltpu.VMEM((2 * C, C), BF16),
            pltpu.VMEM((C, 2 * C), BF16),
            pltpu.VMEM((S, D), BF16),
            pltpu.VMEM((NC, 3, C, D), F32),
            pltpu.VMEM((NC, 3, C, D), F32),
            pltpu.VMEM((2, 2 * C, D), BF16),
            pltpu.VMEM((S, D), F32),
            pltpu.VMEM((5, 8, D), F32),
            pltpu.VMEM((S, D), BF16),
            pltpu.SemaphoreType.DMA((n_dma,)),
        ],
        compiler_params=pltpu.CompilerParams(vmem_limit_bytes=120 * 2**20),
    )(A_q, A_k, A_v, A_shift_k, A_ssm_k, A_ssm_D.reshape(1, D), B_w_gate, B_w_up, B_w_down,
      c, w_mod, jnp.asarray(_FWD, BF16), jnp.asarray(_INV, BF16))
```

```python
import jax
import jax.numpy as jnp
import numpy as np
from jax.experimental import pallas as pl
from jax.experimental.pallas import tpu as pltpu

S, D, F, KS = 2048, 640, 1536, 4
C = 128
NC = S // C
MB = 256
NB = S // MB
EPS = 1e-5
F32 = jnp.float32
BF16 = jnp.bfloat16

FB = 256
CONV_WIN = [-1,-1,-1,-1,2,3,4,5]
MAC_WIN = [-1]*10+[0,1,2,3,4,5]
PRO_CHAIN = [0]*8
LN_ROWS = 16
LN_PAR = [0,2,2,2,2,2,2,2]
LN_PRO = 2
KV_PAR = 2
MAC_PAR = [1]*8
XD = [0]*8
XI = [(6,12)]*8
XO = [3]*8
XW = [2,5,2,2,2,2,2,2]
NWIN = 8


def _dft_matrices():
    n = np.arange(C, dtype=np.float64)
    k = np.concatenate([np.arange(0, C, 2), np.arange(1, C, 2)]).astype(np.float64)
    theta = np.pi * np.outer(2.0 * k + 1.0, n) / (2.0 * C)
    fwd = np.concatenate([np.cos(theta), -np.sin(theta)], axis=0)
    inv = fwd.T / C
    return fwd.astype(np.float32), np.ascontiguousarray(inv).astype(np.float32)


_FWD, _INV = _dft_matrices()


def _layernorm(x):
    m = jnp.mean(x, axis=-1, keepdims=True)
    d = x - m
    v = jnp.mean(d * d, axis=-1, keepdims=True)
    return d * jax.lax.rsqrt(v + EPS)


def _kernel(z_ref, q_hbm, k_hbm, v_hbm, sk_hbm, ssm_hbm, sd_hbm, wg_hbm, wu_hbm, wd_hbm, c_hbm, wm_hbm,
            fwd_hbm, inv_hbm,
            out_hbm,
            q_v, k_v, v_v, sk_v, ssm_v, sd_v, wg_v, wu_v, wd_v, c_v, wm_v, fwd_v, inv_v,
            kv_v, y_v, mod_v, o_v, sems, *spec):
    a_b, kf_b = spec[:NB], spec[NB:]
    z = z_ref[0]
    never = jnp.broadcast_to(z != 0, (8, 128))

    def tie(x, tok):
        return x if tok is None else jnp.where(never, tok, x)

    copies = {}

    def plan(name, src, dst):
        copies[name] = pltpu.make_async_copy(src, dst, sems.at[len(copies)])

    def plan_block(j):
        r = pl.ds(j * MB, MB)
        plan(("k", j), k_hbm.at[0, r, :], k_v.at[r, :])
        plan(("v", j), v_hbm.at[0, r, :], v_v.at[r, :])
        plan(("s", j), ssm_hbm.at[:, r], ssm_v.at[:, r])

    def plan_q(j):
        r = pl.ds(j * MB, MB)
        plan(("q", j), q_hbm.at[0, r, :], q_v.at[r, :])

    plan("fwd", fwd_hbm, fwd_v)
    plan("sk", sk_hbm, sk_v)
    plan("inv", inv_hbm, inv_v)
    plan("sd", sd_hbm, sd_v)
    plan("c", c_hbm, c_v)
    for b in range(NB):
        plan_block(b)
    plan("wmA", wm_hbm.at[:, pl.ds(0, 5 * D)], wm_v.at[:, pl.ds(0, 5 * D)])
    plan("q0", q_hbm.at[0, pl.ds(0, MB), :], q_v.at[pl.ds(0, MB), :])
    plan("wg", wg_hbm, wg_v)
    plan("wu", wu_hbm, wu_v)
    plan("q1", q_hbm.at[0, pl.ds(MB, MB), :], q_v.at[pl.ds(MB, MB), :])
    plan("wd", wd_hbm, wd_v)
    plan("wmB", wm_hbm.at[:, pl.ds(5 * D, D)], wm_v.at[:, pl.ds(5 * D, D)])
    plan("q2", q_hbm.at[0, pl.ds(2 * MB, S - 2 * MB), :], q_v.at[pl.ds(2 * MB, S - 2 * MB), :])
    fs = list(range(0, F, FB))
    n_in = len(copies)
    for cp in copies.values():
        cp.start()
    out_copies = [
        pltpu.make_async_copy(o_v.at[pl.ds(j * MB, MB), :], out_hbm.at[0, pl.ds(j * MB, MB), :],
                              sems.at[n_in + j])
        for j in range(NB)
    ]
    waited = set()

    def wait(*names):
        for nm in names:
            if nm not in waited:
                waited.add(nm)
                copies[nm].wait()

    wait("fwd", "sk", "inv", "sd")
    skt = sk_v[...].astype(F32)
    tap = [jnp.broadcast_to(skt[j:j + 1, :], (8, D)) for j in range(KS)]
    sd = jnp.broadcast_to(sd_v[...].astype(F32).reshape(1, D), (8, D))
    lanes = [slice(l, l + 128) for l in range(0, D, 128)]

    def kv_chunks(cs):
        toks = [None] * KV_PAR
        outs = {}
        n = 0
        for c in cs:
            r0 = c * C
            if c == 0:
                x = jnp.concatenate([jnp.zeros((16, D), F32), k_v[0:C, :].astype(F32)], axis=0)
            else:
                x = k_v[r0 - 16:r0 + C, :].astype(F32)
            sh = [x] + [pltpu.roll(x, j, 0) for j in range(1, KS)]
            vv = v_v[r0:r0 + C, :].astype(F32)
            rows = []
            for r in range(0, C, 8):
                cols = []
                for ls in lanes:
                    t = n % KV_PAR
                    n += 1
                    ks = tie(sh[0][16 + r:24 + r, ls], toks[t]) * tap[0][:, ls]
                    for j in range(1, KS):
                        ks = ks + sh[j][16 + r:24 + r, ls] * tap[j][:, ls]
                    kv = ks * vv[r:r + 8, ls]
                    toks[t] = kv
                    cols.append(kv)
                rows.append(jnp.concatenate(cols, axis=1))
            kv = jnp.concatenate(rows, axis=0).astype(BF16)
            kv_v[r0:r0 + C, :] = kv
            outs[c] = kv
        return outs

    def signal_dft(c, kv):
        a = jnp.dot(fwd_v[...], kv, preferred_element_type=F32)
        a_b[c // 2][c % 2] = a

    prev = [None]

    def filter_dft(p):
        g = jax.lax.dot_general(fwd_v[...], ssm_v[:, p * C:(p + 1) * C], (((1,), (1,)), ((), ())),
                                preferred_element_type=F32)
        re, im = g[:C], g[C:]
        if prev[0] is not None:
            pre, pim = prev[0]
            h = C // 2
            re = jnp.concatenate([re[:h] - pim[:h], re[h:] + pim[h:]], axis=0)
            im = jnp.concatenate([im[:h] + pre[:h], im[h:] - pre[h:]], axis=0)
        kf_b[p // 2][p % 2, 0:C] = re
        kf_b[p // 2][p % 2, C:2 * C] = im
        prev[0] = (g[:C], g[C:])

    def mac_chain(cs, rws):
        tok = (None, None)
        out = {}
        for c in cs:
            for r in rws:
                re_cols, im_cols = [], []
                for l in range(0, D, 128):
                    zr = zi = None
                    for p in range(c + 1):
                        kr = kf_b[p // 2][z + p % 2, r:r + 8, l:l + 128]
                        ki = kf_b[p // 2][z + p % 2, C + r:C + r + 8, l:l + 128]
                        ar = a_b[(c - p) // 2][z + (c - p) % 2, r:r + 8, l:l + 128]
                        ai = a_b[(c - p) // 2][z + (c - p) % 2, C + r:C + r + 8, l:l + 128]
                        if p == 0:
                            kr = tie(kr, tok[0])
                            ki = tie(ki, tok[1])
                            zr = kr * ar - ki * ai
                            zi = kr * ai + ki * ar
                        else:
                            zr = zr + kr * ar
                            zr = zr - ki * ai
                            zi = zi + kr * ai
                            zi = zi + ki * ar
                    tok = (zr, zi)
                    re_cols.append(zr)
                    im_cols.append(zi)
                out[c, r] = (jnp.concatenate(re_cols, axis=1), jnp.concatenate(im_cols, axis=1))
        return out

    def mac_wide(c0, rws):
        out = {}
        for r in rws:
            acc = [None] * 4
            prev_a = None
            for p in range(c0 + 1, -1, -1):
                kr = kf_b[p // 2][z + p % 2, r:r + 8, :]
                ki = kf_b[p // 2][z + p % 2, C + r:C + r + 8, :]
                i = c0 + 1 - p
                cur = (a_b[i // 2][z + i % 2, r:r + 8, :], a_b[i // 2][z + i % 2, C + r:C + r + 8, :])
                for o, a in ((1, cur), (0, prev_a)):
                    if a is None:
                        continue
                    tr = kr * a[0] - ki * a[1]
                    ti = kr * a[1] + ki * a[0]
                    acc[2 * o] = tr if acc[2 * o] is None else acc[2 * o] + tr
                    acc[2 * o + 1] = ti if acc[2 * o + 1] is None else acc[2 * o + 1] + ti
                prev_a = cur
            out[c0, r] = (acc[0], acc[1])
            out[c0 + 1, r] = (acc[2], acc[3])
        return out

    def mac(cs, nchain):
        rws = list(range(0, C, 8))
        parts = mac_chain(cs, rws[:nchain])
        if nchain < len(rws):
            parts.update(mac_wide(cs[0], rws[nchain:]))
        return {c: jnp.concatenate([parts[c, r][0] for r in rws] + [parts[c, r][1] for r in rws],
                                   axis=0).astype(BF16) for c in cs}

    def inverse_dft(c, w):
        r0 = c * C
        y = jnp.dot(inv_v[...], w, preferred_element_type=F32)
        y_v[r0:r0 + C, :] = y + kv_v[r0:r0 + C, :].astype(F32) * sd[0:1]

    def ln_block(j, par):
        r0 = j * MB
        toks = [None] * par
        xs, hs = [], []
        n = 0
        for r in range(0, MB, 16):
            q16 = q_v[r0 + r:r0 + r + 16, :].astype(F32)
            hh = []
            for g in (0, 8):
                t = n % par
                n += 1
                qq = q16[g:g + 8]
                qq = jnp.concatenate([tie(qq[:, 0:128], toks[t]), qq[:, 128:]], axis=1)
                x = qq + y_v[r0 + r + g:r0 + r + g + 8, :] * (_layernorm(qq) * mod_v[0] + mod_v[1])
                h = _layernorm(x) * mod_v[2] + mod_v[3]
                toks[t] = h[:, 0:128]
                xs.append(x)
                hh.append(h)
            hs.append(jnp.concatenate(hh, axis=0).astype(BF16))
        return jnp.concatenate(xs, axis=0), jnp.concatenate(hs, axis=0)

    def conv_front(b):
        wait(("k", b), ("v", b), ("s", b))
        return kv_chunks((2 * b, 2 * b + 1))

    def conv_dft(b, kv):
        for c in (2 * b, 2 * b + 1):
            signal_dft(c, kv[c])
            filter_dft(c)

    def mac_block(b, ribbon=True):
        return mac((2 * b, 2 * b + 1), MAC_PAR[b] if ribbon else 64)

    def idft_block(b, w):
        for c in (2 * b, 2 * b + 1):
            inverse_dft(c, w[c])

    def finish(j, x, acc):
        o_v[j * MB:(j + 1) * MB, :] = (x + acc * mod_v[4, 0:1]).astype(BF16)
        out_copies[j].start()

    ws = {}
    for b in range(NB + 1):
        if b < NB:
            wait(("k", b), ("v", b), ("s", b))
        if b < NB:
            conv_dft(b, kv_chunks((2 * b, 2 * b + 1)))
        for c in list(ws):
            inverse_dft(c, ws.pop(c))
        if b >= 1 and MAC_WIN[2 * b - 1] < 0:
            ws.update(mac((2 * b - 2, 2 * b - 1), PRO_CHAIN[b - 1]))
    for c in list(ws):
        inverse_dft(c, ws.pop(c))

    wait("c", "wmA", "q0")
    cc = c_v[...].astype(F32)
    sc = jnp.broadcast_to((cc * jax.nn.sigmoid(cc)).astype(BF16), (16, D))
    mod = jnp.dot(sc, wm_v[:, 0:5 * D], preferred_element_type=F32)[0:8]
    sa, ca, ga, sb, cb = (mod[:, i * D:(i + 1) * D] for i in range(5))
    mod_v[0] = ga * (1.0 + ca)
    mod_v[1] = ga * sa
    mod_v[2] = 1.0 + cb
    mod_v[3] = sb

    xh = {}
    xh[0] = ln_block(0, 64)

    pend = None
    for j in range(NWIN):
        x, h = xh.pop(j)
        steps = []
        for i, f in enumerate(fs):
            steps.append(("gu", f))
            if i > 0:
                steps.append(("dn", fs[i - 1]))
        steps.append(("dn", fs[-1]))
        ws = {}

        def side_work():
            for c in range(NC):
                if MAC_WIN[c] == j:
                    ws.update(mac((c,), 16))
            if j + 1 < NB:
                xh[j + 1] = ln_block(j + 1, LN_PAR[j + 1])

        if j == 0:
            steps = [("gu", f) for f in fs] + [("mid", 0)] + [("dn", f) for f in fs]
            wait("wg", "wu")
        else:
            if j == 1:
                wait(*copies)
                mod_v[4] = jnp.dot(sc, wm_v[:, 5 * D:], preferred_element_type=F32)[0:8]
            side_work()
        hh = {}
        acc = None
        for kind, f in steps:
            if kind == "mid":
                wait("q1", "wd")
                side_work()
            elif kind == "gu":
                g = jnp.dot(h, wg_v[:, f:f + FB], preferred_element_type=F32)
                u = jnp.dot(h, wu_v[:, f:f + FB], preferred_element_type=F32)
                hh[f] = (g * u).astype(BF16)
            else:
                t = jnp.dot(hh.pop(f), wd_v[f:f + FB, :], preferred_element_type=F32)
                acc = t if acc is None else acc + t
        for c in list(ws):
            inverse_dft(c, ws.pop(c))
        if pend is not None:
            finish(*pend)
        pend = (j, x, acc)
    finish(*pend)
    for j in range(NWIN - 1):
        out_copies[j].wait()
    out_copies[NWIN - 1].wait()
    for nm in copies:
        wait(nm)


@jax.jit
def pallas_adaLN_cond__ssm_conv_h3__glu_gated_bilinear__prompt_kernel(
    A_q, A_k, A_v, A_shift_k, A_ssm_k, A_ssm_D, B_x, B_w_gate, B_w_up, B_w_down, c, w_mod,
):
    del B_x
    any_spec = pl.BlockSpec(memory_space=pl.ANY)
    n_dma = 5 + 3 * NB + 8 + NB
    return pl.pallas_call(
        _kernel,
        out_shape=jax.ShapeDtypeStruct((1, S, D), BF16),
        in_specs=[pl.BlockSpec(memory_space=pltpu.SMEM)] + [any_spec] * 13,
        out_specs=any_spec,
        scratch_shapes=[
            pltpu.VMEM((S, D), BF16),
            pltpu.VMEM((S, D), BF16),
            pltpu.VMEM((S, D), BF16),
            pltpu.VMEM((KS, D), BF16),
            pltpu.VMEM((D, S), BF16),
            pltpu.VMEM((D,), BF16),
            pltpu.VMEM((D, F), BF16),
            pltpu.VMEM((D, F), BF16),
            pltpu.VMEM((F, D), BF16),
            pltpu.VMEM((1, D), BF16),
            pltpu.VMEM((D, 6 * D), BF16),
            pltpu.VMEM((2 * C, C), BF16),
            pltpu.VMEM((C, 2 * C), BF16),
            pltpu.VMEM((S, D), BF16),
            pltpu.VMEM((S, D), F32),
            pltpu.VMEM((5, 8, D), F32),
            pltpu.VMEM((S, D), BF16),
            pltpu.SemaphoreType.DMA((n_dma,)),
        ] + [pltpu.VMEM((2, 2 * C, D), F32)] * (2 * NB),
        compiler_params=pltpu.CompilerParams(vmem_limit_bytes=120 * 2**20),
    )(jnp.zeros((1,), jnp.int32), A_q, A_k, A_v, A_shift_k.T, A_ssm_k, A_ssm_D, B_w_gate, B_w_up,
      B_w_down, c, w_mod, jnp.asarray(_FWD, BF16), jnp.asarray(_INV, BF16))
```
